```python
import os as _os
_os.environ.setdefault("JAX_PLATFORMS", "cpu")
import jax
import jax.numpy as jnp

def _softmax(x, axis=-1):
    return jax.nn.softmax(x, axis=axis)
def _gelu(x):
    return jax.nn.gelu(x, approximate=True)
def _silu(x):
    return jax.nn.silu(x)
def _sigmoid(x):
    return jax.nn.sigmoid(x)
def _layernorm(x, axis=-1, eps=1e-5):
    m = jnp.mean(x, axis=axis, keepdims=True)
    v = jnp.var(x, axis=axis, keepdims=True)
    return (x - m) / jnp.sqrt(v + eps)
def _scatter_add(tgt, idx, src, axis=0):
    return tgt.at[idx].add(src)
def _segment_sum(src, seg, n):
    return jax.ops.segment_sum(src, seg, n)
class _Rng:
    def __init__(self, key):
        self._k = key
    def _next(self):
        self._k, sub = jax.random.split(self._k)
        return sub
    def normal(self, shape):
        return jax.random.normal(self._next(), shape, dtype=jnp.bfloat16)
    def randint(self, lo, hi, shape):
        return jax.random.randint(self._next(), shape, lo, hi, dtype=jnp.int32)
    def uniform(self, shape, lo=0.0, hi=1.0):
        return jax.random.uniform(self._next(), shape, jnp.bfloat16, lo, hi)
    def permutation(self, n):
        return jax.random.permutation(self._next(), n)


kernel_name = 'standalone__mha_softmax__sampling'

def setup_inputs():
    _rng = _Rng(jax.random.key(int.from_bytes(__import__("os").urandom(4), "little")))
    _w = (lambda a: (lambda t: t.astype(jnp.bfloat16) if jnp.issubdtype(t.dtype, jnp.floating) else t)(jnp.asarray(a)))
    B, H, Sq, Sk, D = 8, 32, 32, 2048, 128
    return {
        "q": _w((lambda *s: _rng.normal(s) * 0.4)(B, H, Sq, D)),
        "k": _w((lambda *s: _rng.normal(s) * 0.4)(B, H, Sk, D)),
        "v": _w((lambda *s: _rng.normal(s) * 0.05)(B, H, Sk, D)),
    }

def reference(q, k, v):
    scale = q.shape[-1] ** -0.5
    scores = jnp.einsum("bhqd,bhkd->bhqk", q, k) * scale
    p = _softmax(scores, axis=-1)
    return jnp.einsum("bhqk,bhkd->bhqd", p, v)
```

```python
import jax
import jax.numpy as jnp
import jax.experimental.pallas as pl
import jax.experimental.pallas.tpu as pltpu

_DEPTH = 6
_KV_PIECES = 11
_QO_PIECES = 46
_Q_HEAD_START = 4
_O_TAIL = 2
_ROW_TILE = 16


def _split(rows, n):
    units = rows // _ROW_TILE
    n = max(1, min(n, units))
    sizes = [(units // n + (1 if j < units % n else 0)) * _ROW_TILE for j in range(n)]
    sizes[-1] += rows - sum(sizes)
    starts = [sum(sizes[:j]) for j in range(n)]
    return list(zip(starts, sizes))


def _mha_kernel(q_hbm, k_hbm, v_hbm, o_hbm, qbuf, kbuf, vbuf, obuf, qsem, ksem, vsem, osem):
    n_heads, sk, d = k_hbm.shape
    sq = q_hbm.shape[0] // n_heads
    depth = kbuf.shape[0]
    scale = d ** -0.5

    def start_kv(h, slot):
        for r, m in _split(sk, _KV_PIECES):
            rows = pl.ds(r, m)
            pltpu.make_async_copy(k_hbm.at[h, rows], kbuf.at[slot, rows], ksem.at[slot]).start(priority=0)
            pltpu.make_async_copy(v_hbm.at[h, rows], vbuf.at[slot, rows], vsem.at[slot]).start(priority=1)

    def start_heads(src, dst, sem, h0, h1, pieces):
        for j, (r, m) in enumerate(_split((h1 - h0) * sq, pieces)):
            rows = pl.ds(h0 * sq + r, m)
            pltpu.make_async_copy(src.at[rows], dst.at[rows], sem).start(priority=j % 2)

    def wait_heads(buf, sem, h0, h1):
        rows = pl.ds(h0 * sq, (h1 - h0) * sq)
        pltpu.make_async_copy(buf.at[rows], buf.at[rows], sem).wait()

    start_heads(q_hbm, qbuf, qsem.at[0], 0, _Q_HEAD_START, 1)
    for slot in range(depth):
        if slot == 1:
            start_heads(q_hbm, qbuf, qsem.at[1], _Q_HEAD_START, n_heads, _QO_PIECES)
        start_kv(slot, slot)
    wait_heads(qbuf, qsem.at[0], 0, _Q_HEAD_START)

    def body(h, carry):
        slot = h % depth
        rows = pl.ds(pl.multiple_of(h * sq, sq), sq)

        @pl.when(h == _Q_HEAD_START)
        def _():
            wait_heads(qbuf, qsem.at[1], _Q_HEAD_START, n_heads)

        pltpu.make_async_copy(kbuf.at[slot], kbuf.at[slot], ksem.at[slot]).wait()

        @pl.when(h == n_heads - _O_TAIL)
        def _():
            start_heads(obuf, o_hbm, osem.at[0], 0, n_heads - _O_TAIL, _QO_PIECES)

        s = jax.lax.dot_general(
            qbuf[rows], kbuf[slot], (((1,), (1,)), ((), ())), preferred_element_type=jnp.float32
        ) * scale
        p = jnp.exp(s - jnp.max(s, axis=-1, keepdims=True))
        denom = jnp.sum(p, axis=-1, keepdims=True)

        pltpu.make_async_copy(vbuf.at[slot], vbuf.at[slot], vsem.at[slot]).wait()
        o = jnp.dot(p.astype(vbuf.dtype), vbuf[slot], preferred_element_type=jnp.float32)
        obuf[rows] = (o / denom).astype(obuf.dtype)

        @pl.when(h + depth < n_heads)
        def _():
            start_kv(h + depth, slot)

        return carry

    jax.lax.fori_loop(0, n_heads, body, None)
    start_heads(obuf, o_hbm, osem.at[0], n_heads - _O_TAIL, n_heads, _O_TAIL)
    wait_heads(obuf, osem.at[0], 0, n_heads)


@jax.jit
def pallas_standalone__mha_softmax__sampling_kernel(
    q: jax.Array,
    k: jax.Array,
    v: jax.Array,
):
    b, h, sq, d = q.shape
    sk = k.shape[2]
    n = b * h
    out = pl.pallas_call(
        _mha_kernel,
        in_specs=[pl.BlockSpec(memory_space=pl.ANY)] * 3,
        out_specs=pl.BlockSpec(memory_space=pl.ANY),
        out_shape=jax.ShapeDtypeStruct((n * sq, d), q.dtype),
        scratch_shapes=[
            pltpu.VMEM((n * sq, d), q.dtype),
            pltpu.VMEM((_DEPTH, sk, d), k.dtype),
            pltpu.VMEM((_DEPTH, sk, d), v.dtype),
            pltpu.VMEM((n * sq, d), q.dtype),
            pltpu.SemaphoreType.DMA((2,)),
            pltpu.SemaphoreType.DMA((_DEPTH,)),
            pltpu.SemaphoreType.DMA((_DEPTH,)),
            pltpu.SemaphoreType.DMA((1,)),
        ],
        compiler_params=pltpu.CompilerParams(vmem_limit_bytes=64 * 2**20),
    )(q.reshape(n * sq, d), k.reshape(n, sk, d), v.reshape(n, sk, d))
    return out.reshape(b, h, sq, d)
```

```python
import math

import jax
import jax.numpy as jnp
import jax.experimental.pallas as pl
import jax.experimental.pallas.tpu as pltpu

_LANES = 6
_STRIDE = 2
_SLOTS = 3
_AHEAD = 2
_PIECES = 72
_TAIL_PIECES = 18
_TAIL_MIN_ROWS = 6
_OUT_PIECES = 24
_UNROLL = 2
_ROW_TILE = 16


def _split(rows, n):
    units = max(1, rows // _ROW_TILE)
    n = max(1, min(n, units))
    sizes = [(units // n + (1 if j < units % n else 0)) * _ROW_TILE for j in range(n)]
    sizes[-1] += rows - sum(sizes)
    return [(sum(sizes[:j]), m) for j, m in enumerate(sizes)]


def _share(pieces, j, n):
    return pieces[j * len(pieces) // n:(j + 1) * len(pieces) // n]


def _plan(n_rows):
    main_rows = max(0, n_rows - _TAIL_MIN_ROWS) // _LANES * _LANES
    tail, step, row = [], main_rows * _STRIDE, main_rows
    while row < n_rows:
        left = n_rows - row
        lanes = min(4, left - 4) if left > 4 else min(2, left)
        for phase in range(_STRIDE):
            tail.append((step, lanes, row, phase))
            step += lanes
        row += lanes
    return main_rows * _STRIDE, tail


def _mha_kernel(q_hbm, k_hbm, v_hbm, o_hbm, qbuf, kbuf, vbuf, obuf, qsem, ksem, vsem, osem):
    n_rows, _, sk, d = k_hbm.shape
    sq = q_hbm.shape[2]
    n_heads = n_rows * _STRIDE
    n_main, tail = _plan(n_rows)
    ring = _SLOTS * _LANES
    lookahead = _LANES + _AHEAD
    exp2_scale = d ** -0.5 * math.log2(math.e)

    def start_q(row, lanes, phase, pos, sem):
        pltpu.make_async_copy(
            q_hbm.at[pl.ds(row, lanes), phase], qbuf.at[pl.ds(pos, lanes)], qsem.at[sem]
        ).start(priority=1)

    def start_kv(row, lanes, phase, pos, sem, pieces):
        for r, m in pieces:
            for queue, (src, buf, sems) in enumerate(((k_hbm, kbuf, ksem), (v_hbm, vbuf, vsem))):
                pltpu.make_async_copy(
                    src.at[pl.ds(row, lanes), phase, pl.ds(r, m)],
                    buf.at[pl.ds(pos, lanes), pl.ds(r, m)],
                    sems.at[sem],
                ).start(priority=queue)

    def wait_q(lanes, pos, sem):
        filled = qbuf.at[pl.ds(pos, lanes)]
        pltpu.make_async_copy(filled, filled, qsem.at[sem]).wait()

    def wait_kv(lanes, pos, sem, r0=0, r1=sk):
        for buf, sems in ((kbuf, ksem), (vbuf, vsem)):
            filled = buf.at[pl.ds(pos, lanes), pl.ds(r0, r1 - r0)]
            pltpu.make_async_copy(filled, filled, sems.at[sem]).wait()

    def start_main_slice(row, phase, slot, lane):
        if lane == 0:
            start_q(row, _LANES, phase, slot * _LANES, slot)
        start_kv(row, _LANES, phase, slot * _LANES, slot, _share(_split(sk, _PIECES), lane, _LANES))

    last_pieces = _split(sk, _TAIL_PIECES * tail[-1][1])
    cue_rows = last_pieces[len(last_pieces) // 2][0]
    cue_sem = _SLOTS + len(tail)

    def start_tail_slice(t, lane):
        step, lanes, row, phase = tail[t]
        pos = ring + step - n_main
        if lane == 0:
            start_q(row, lanes, phase, pos, _SLOTS + t)
        for r, m in _share(_split(sk, _TAIL_PIECES * lanes), lane, lanes):
            cue = t == len(tail) - 1 and r < cue_rows
            start_kv(row, lanes, phase, pos, cue_sem if cue else _SLOTS + t, [(r, m)])

    def start_output(h0, h1, n):
        pieces = _split((h1 - h0) * sq, n)
        streams = [_share(pieces, j, 4) for j in range(4)]
        for i in range(max(len(s) for s in streams)):
            for j, stream in enumerate(streams):
                if i < len(stream):
                    rows = pl.ds(h0 * sq + stream[i][0], stream[i][1])
                    pltpu.make_async_copy(obuf.at[rows], o_hbm.at[rows], osem.at[0]).start(priority=j % 2)

    tail_starts, at = [], n_main - 1 - lookahead
    for t, (step, lanes, _, _) in enumerate(tail):
        for lane in range(lanes):
            j = step + lane - _AHEAD
            waited_lanes = ([_LANES] + [g[1] for g in tail if g[0] <= j])[-1]
            at = min(max(at + 1, j - waited_lanes), step)
            tail_starts.append((at, t, lane))

    for j in range(min(lookahead, n_main)):
        group = j // _LANES
        start_main_slice(group // _STRIDE * _LANES, group % _STRIDE, group % _SLOTS, j % _LANES)
    for at, t, lane in tail_starts:
        if at < 0:
            start_tail_slice(t, lane)

    def div(a, b):
        return lax_div(a, jnp.int32(b))

    def rem(a, b):
        return lax_rem(a, jnp.int32(b))

    lax_div, lax_rem = jax.lax.div, jax.lax.rem

    def advance(step):
        j = step + lookahead
        next_group, next_lane = div(j, _LANES), rem(j, _LANES)
        for lane in range(_LANES):
            @pl.when(jnp.logical_and(j < n_main, next_lane == lane))
            def _():
                start_main_slice(
                    div(next_group, _STRIDE) * _LANES, rem(next_group, _STRIDE), rem(next_group, _SLOTS), lane
                )

        group = div(step, _LANES)

        @pl.when(jnp.logical_and(step < n_main, rem(step, _LANES) == 0))
        def _():
            slot = rem(group, _SLOTS)
            wait_q(_LANES, slot * _LANES, slot)
            wait_kv(_LANES, slot * _LANES, slot)

        @pl.when(j >= n_main)
        def _():
            for at, t, lane in tail_starts:
                if at >= 0:
                    @pl.when(step == at)
                    def _():
                        start_tail_slice(t, lane)
            for t, (first, lanes, _, _) in enumerate(tail):
                @pl.when(step == first)
                def _():
                    pos = ring + first - n_main
                    wait_q(lanes, pos, _SLOTS + t)
                    if t < len(tail) - 1:
                        wait_kv(lanes, pos, _SLOTS + t)
                        return
                    if cue_rows:
                        wait_kv(lanes, pos, cue_sem, 0, cue_rows)
                    if n_main:
                        start_output(0, n_main, _OUT_PIECES)
                    wait_kv(lanes, pos, _SLOTS + t, cue_rows, sk)

        pos = jnp.where(step < n_main, rem(step, ring), ring + step - n_main)
        head = (div(group, _STRIDE) * _LANES + rem(step, _LANES)) * _STRIDE + rem(group, _STRIDE)
        for first, _, row, phase in tail:
            head = jnp.where(step >= first, (row + step - first) * _STRIDE + phase, head)
        return pos, head

    def body(i, carry):
        due = [advance(i * _UNROLL + u) for u in range(_UNROLL)]
        for pos, head in due:
            s = jax.lax.dot_general(
                qbuf[pos], kbuf[pos], (((1,), (1,)), ((), ())), preferred_element_type=jnp.float32
            )
            p = jnp.exp2((s - jnp.max(s, axis=-1, keepdims=True)) * exp2_scale)
            denom = jnp.sum(p, axis=-1, keepdims=True)
            o = jnp.dot(p.astype(vbuf.dtype), vbuf[pos], preferred_element_type=jnp.float32)
            obuf[pl.ds(pl.multiple_of(head * sq, sq), sq)] = (o / denom).astype(obuf.dtype)
        return carry

    jax.lax.fori_loop(0, n_heads // _UNROLL, body, None)
    start_output(n_main, n_heads, 2)
    pltpu.make_async_copy(obuf, o_hbm, osem.at[0]).wait()


@jax.jit
def pallas_standalone__mha_softmax__sampling_kernel(
    q: jax.Array,
    k: jax.Array,
    v: jax.Array,
):
    b, h, sq, d = q.shape
    sk = k.shape[2]
    n_heads = b * h
    assert n_heads % _STRIDE == 0 and n_heads % _UNROLL == 0
    n_rows = n_heads // _STRIDE
    n_main, tail = _plan(n_rows)
    positions = _SLOTS * _LANES + n_heads - n_main
    n_sems = _SLOTS + len(tail) + 1
    out = pl.pallas_call(
        _mha_kernel,
        in_specs=[pl.BlockSpec(memory_space=pl.ANY)] * 3,
        out_specs=pl.BlockSpec(memory_space=pl.ANY),
        out_shape=jax.ShapeDtypeStruct((n_heads * sq, d), q.dtype),
        scratch_shapes=[
            pltpu.VMEM((positions, sq, d), q.dtype),
            pltpu.VMEM((positions, sk, d), k.dtype),
            pltpu.VMEM((positions, sk, d), v.dtype),
            pltpu.VMEM((n_heads * sq, d), q.dtype),
            pltpu.SemaphoreType.DMA((n_sems,)),
            pltpu.SemaphoreType.DMA((n_sems,)),
            pltpu.SemaphoreType.DMA((n_sems,)),
            pltpu.SemaphoreType.DMA((1,)),
        ],
        compiler_params=pltpu.CompilerParams(vmem_limit_bytes=64 * 2**20),
    )(
        q.reshape(n_rows, _STRIDE, sq, d),
        k.reshape(n_rows, _STRIDE, sk, d),
        v.reshape(n_rows, _STRIDE, sk, d),
    )
    return out.reshape(b, h, sq, d)
```

```python
import math

import jax
import jax.numpy as jnp
import jax.experimental.pallas as pl
import jax.experimental.pallas.tpu as pltpu

_LANES = 6
_STRIDE = 2
_SLOTS = 3
_AHEAD = 3
_PIECES = 72
_TAIL_PIECES = 18
_TAIL_MIN_ROWS = 6
_OUT_LANES = 4
_OUT_ROWS = 48
_UNROLL = 4
_ROW_TILE = 16


def _split(rows, n):
    units = max(1, rows // _ROW_TILE)
    n = max(1, min(n, units))
    sizes = [(units // n + (1 if j < units % n else 0)) * _ROW_TILE for j in range(n)]
    sizes[-1] += rows - sum(sizes)
    return [(sum(sizes[:j]), m) for j, m in enumerate(sizes)]


def _share(pieces, j, n):
    return pieces[j * len(pieces) // n:(j + 1) * len(pieces) // n]


def _plan(n_rows):
    main_rows = max(0, n_rows - _TAIL_MIN_ROWS) // _LANES * _LANES
    tail, step, row = [], main_rows * _STRIDE, main_rows
    while row < n_rows:
        left = n_rows - row
        lanes = min(4, left - 4) if left > 4 else min(2, left)
        for phase in range(_STRIDE):
            tail.append((step, lanes, row, phase))
            step += lanes
        row += lanes
    return main_rows * _STRIDE, tail


def _mha_kernel(q_hbm, k_hbm, v_hbm, o_hbm, qbuf, kbuf, vbuf, obuf, qsem, ksem, vsem, osem):
    n_rows, _, sk, d = k_hbm.shape
    sq = q_hbm.shape[2]
    n_heads = n_rows * _STRIDE
    n_main, tail = _plan(n_rows)
    ring = _SLOTS * _LANES
    lookahead = _LANES + _AHEAD
    exp2_scale = d ** -0.5 * math.log2(math.e)

    def start_q(row, lanes, phase, pos, sem):
        pltpu.make_async_copy(
            q_hbm.at[pl.ds(row, lanes), phase], qbuf.at[pl.ds(pos, lanes)], qsem.at[sem]
        ).start(priority=1)

    def start_kv(row, lanes, phase, pos, sem, pieces):
        for r, m in pieces:
            for queue, (src, buf, sems) in enumerate(((k_hbm, kbuf, ksem), (v_hbm, vbuf, vsem))):
                pltpu.make_async_copy(
                    src.at[pl.ds(row, lanes), phase, pl.ds(r, m)],
                    buf.at[pl.ds(pos, lanes), pl.ds(r, m)],
                    sems.at[sem],
                ).start(priority=queue)

    def wait_q(lanes, pos, sem):
        filled = qbuf.at[pl.ds(pos, lanes)]
        pltpu.make_async_copy(filled, filled, qsem.at[sem]).wait()

    def wait_kv(lanes, pos, sem, r0=0, r1=sk):
        for buf, sems in ((kbuf, ksem), (vbuf, vsem)):
            filled = buf.at[pl.ds(pos, lanes), pl.ds(r0, r1 - r0)]
            pltpu.make_async_copy(filled, filled, sems.at[sem]).wait()

    def start_main_slice(row, phase, slot, lane):
        if lane == 0:
            start_q(row, _LANES, phase, slot * _LANES, slot)
        start_kv(row, _LANES, phase, slot * _LANES, slot, _share(_split(sk, _PIECES), lane, _LANES))

    last_pieces = _split(sk, _TAIL_PIECES * tail[-1][1])
    cue_rows = last_pieces[len(last_pieces) // 2][0]
    cue_sem = _SLOTS + len(tail)

    def start_tail_slice(t, lane):
        step, lanes, row, phase = tail[t]
        pos = ring + step - n_main
        if lane == 0:
            start_q(row, lanes, phase, pos, _SLOTS + t)
        for r, m in _share(_split(sk, _TAIL_PIECES * lanes), lane, lanes):
            cue = t == len(tail) - 1 and r < cue_rows
            start_kv(row, lanes, phase, pos, cue_sem if cue else _SLOTS + t, [(r, m)])

    def start_output(lanes, rows, queue):
        pltpu.make_async_copy(obuf.at[lanes, rows], o_hbm.at[lanes, rows], osem.at[0]).start(priority=queue)

    part_heads = n_heads // _OUT_LANES
    part_rows = part_heads * sq
    bulk_rows = n_main * sq - (_OUT_LANES - 1) * part_rows

    def start_bulk_output():
        todo = [(r, m, _OUT_LANES) for r, m in _split(bulk_rows, bulk_rows // _OUT_ROWS)]
        rest = part_rows - bulk_rows
        todo += [(bulk_rows + r, m, _OUT_LANES - 1) for r, m in _split(rest, rest // _OUT_ROWS)]
        half = (len(todo) + 1) // 2
        for i in range(half):
            for queue, (r, m, lanes) in enumerate(todo[i:i + 1] + todo[half + i:half + i + 1]):
                start_output(pl.ds(0, lanes), pl.ds(r, m), queue)

    tail_starts, at = [], n_main - 1 - lookahead
    for t, (step, lanes, _, _) in enumerate(tail):
        for lane in range(lanes):
            j = step + lane - _AHEAD
            waited_lanes = ([_LANES] + [g[1] for g in tail if g[0] <= j])[-1]
            at = min(max(at + 1, j - waited_lanes), step)
            tail_starts.append((at, t, lane))

    for j in range(min(lookahead, n_main)):
        group = j // _LANES
        start_main_slice(group // _STRIDE * _LANES, group % _STRIDE, group % _SLOTS, j % _LANES)
    for at, t, lane in tail_starts:
        if at < 0:
            start_tail_slice(t, lane)

    def div(a, b):
        return jax.lax.div(a, jnp.int32(b))

    def rem(a, b):
        return jax.lax.rem(a, jnp.int32(b))

    assert all((g * _LANES - lookahead) // _UNROLL * _UNROLL >= (g - _SLOTS + 1) * _LANES
               for g in range(_SLOTS, n_main // _LANES))
    assert tail[-1][0] // _UNROLL * _UNROLL >= n_main

    def advance(step, carry):
        j = step + lookahead
        next_group, next_lane = div(j, _LANES), rem(j, _LANES)
        for lane in range(_LANES):
            @pl.when(jnp.logical_and(j < n_main, next_lane == lane))
            def _():
                start_main_slice(
                    div(next_group, _STRIDE) * _LANES, rem(next_group, _STRIDE), rem(next_group, _SLOTS), lane
                )

        @pl.when(jnp.logical_and(step < n_main, rem(step, _LANES) == 0))
        def _():
            slot = rem(div(step, _LANES), _SLOTS)
            wait_q(_LANES, slot * _LANES, slot)
            wait_kv(_LANES, slot * _LANES, slot)

        @pl.when(j >= n_main)
        def _():
            for at, t, lane in tail_starts:
                if at >= 0:
                    @pl.when(step == at)
                    def _():
                        start_tail_slice(t, lane)
            for t, (first, lanes, _, _) in enumerate(tail):
                @pl.when(step == first)
                def _():
                    pos = ring + first - n_main
                    wait_q(lanes, pos, _SLOTS + t)
                    if t < len(tail) - 1:
                        wait_kv(lanes, pos, _SLOTS + t)
                        return
                    if cue_rows:
                        wait_kv(lanes, pos, cue_sem, 0, cue_rows)
                    if bulk_rows > 0:
                        start_bulk_output()
                    wait_kv(lanes, pos, _SLOTS + t, cue_rows, sk)

        return carry

    def locate(step):
        group = div(step, _LANES)
        pos = jnp.where(step < n_main, rem(step, ring), ring + step - n_main)
        head = (div(group, _STRIDE) * _LANES + rem(step, _LANES)) * _STRIDE + rem(group, _STRIDE)
        for first, _, row, phase in tail:
            head = jnp.where(step >= first, (row + step - first) * _STRIDE + phase, head)
        return pos, head

    def body(i, carry):
        jax.lax.fori_loop(i * _UNROLL, (i + 1) * _UNROLL, advance, None)
        for u in range(_UNROLL):
            pos, head = locate(i * _UNROLL + u)
            s = jax.lax.dot_general(
                qbuf[pos], kbuf[pos], (((1,), (1,)), ((), ())), preferred_element_type=jnp.float32
            )
            p = jnp.exp2((s - jnp.max(s, axis=-1, keepdims=True)) * exp2_scale)
            denom = jnp.sum(p, axis=-1, keepdims=True)
            o = jnp.dot(p.astype(vbuf.dtype), vbuf[pos], preferred_element_type=jnp.float32)
            rows = pl.ds(pl.multiple_of(rem(head, part_heads) * sq, sq), sq)
            obuf[div(head, part_heads), rows] = (o / denom).astype(obuf.dtype)
        return carry

    jax.lax.fori_loop(0, n_heads // _UNROLL, body, None)
    if bulk_rows > 0:
        start_output(pl.ds(_OUT_LANES - 1, 1), pl.ds(bulk_rows, part_rows - bulk_rows), 0)
    else:
        start_output(pl.ds(0, _OUT_LANES), pl.ds(0, part_rows), 0)
    pltpu.make_async_copy(obuf, o_hbm, osem.at[0]).wait()


@jax.jit
def pallas_standalone__mha_softmax__sampling_kernel(
    q: jax.Array,
    k: jax.Array,
    v: jax.Array,
):
    b, h, sq, d = q.shape
    sk = k.shape[2]
    n_heads = b * h
    assert n_heads % _STRIDE == 0 and n_heads % _UNROLL == 0 and n_heads % _OUT_LANES == 0
    out_view = (_OUT_LANES, n_heads // _OUT_LANES * sq, d)
    n_rows = n_heads // _STRIDE
    n_main, tail = _plan(n_rows)
    positions = _SLOTS * _LANES + n_heads - n_main
    n_sems = _SLOTS + len(tail) + 1
    out = pl.pallas_call(
        _mha_kernel,
        in_specs=[pl.BlockSpec(memory_space=pl.ANY)] * 3,
        out_specs=pl.BlockSpec(memory_space=pl.ANY),
        out_shape=jax.ShapeDtypeStruct(out_view, q.dtype),
        scratch_shapes=[
            pltpu.VMEM((positions, sq, d), q.dtype),
            pltpu.VMEM((positions, sk, d), k.dtype),
            pltpu.VMEM((positions, sk, d), v.dtype),
            pltpu.VMEM(out_view, q.dtype),
            pltpu.SemaphoreType.DMA((n_sems,)),
            pltpu.SemaphoreType.DMA((n_sems,)),
            pltpu.SemaphoreType.DMA((n_sems,)),
            pltpu.SemaphoreType.DMA((1,)),
        ],
        compiler_params=pltpu.CompilerParams(vmem_limit_bytes=64 * 2**20),
    )(
        q.reshape(n_rows, _STRIDE, sq, d),
        k.reshape(n_rows, _STRIDE, sk, d),
        v.reshape(n_rows, _STRIDE, sk, d),
    )
    return out.reshape(b, h, sq, d)
```
